```python
import os as _os
_os.environ.setdefault("JAX_PLATFORMS", "cpu")
import jax
import jax.numpy as jnp

def _softmax(x, axis=-1):
    return jax.nn.softmax(x, axis=axis)
def _gelu(x):
    return jax.nn.gelu(x, approximate=True)
def _silu(x):
    return jax.nn.silu(x)
def _sigmoid(x):
    return jax.nn.sigmoid(x)
def _layernorm(x, axis=-1, eps=1e-5):
    m = jnp.mean(x, axis=axis, keepdims=True)
    v = jnp.var(x, axis=axis, keepdims=True)
    return (x - m) / jnp.sqrt(v + eps)
def _scatter_add(tgt, idx, src, axis=0):
    return tgt.at[idx].add(src)
def _segment_sum(src, seg, n):
    return jax.ops.segment_sum(src, seg, n)
class _Rng:
    def __init__(self, key):
        self._k = key
    def _next(self):
        self._k, sub = jax.random.split(self._k)
        return sub
    def normal(self, shape):
        return jax.random.normal(self._next(), shape, dtype=jnp.bfloat16)
    def randint(self, lo, hi, shape):
        return jax.random.randint(self._next(), shape, lo, hi, dtype=jnp.int32)
    def uniform(self, shape, lo=0.0, hi=1.0):
        return jax.random.uniform(self._next(), shape, jnp.bfloat16, lo, hi)
    def permutation(self, n):
        return jax.random.permutation(self._next(), n)


kernel_name = 'interleave_layers__linear_attn_block__mha_block__prompt'

def setup_inputs():
    _rng = _Rng(jax.random.key(int.from_bytes(__import__("os").urandom(4), "little")))
    _w = (lambda a: (lambda t: t.astype(jnp.bfloat16) if jnp.issubdtype(t.dtype, jnp.floating) else t)(jnp.asarray(a)))
    def _A_setup():
        B, S, D = 1, 2048, 640
        return {
            "x": _w((lambda *s: _rng.normal(s) * 0.05)(B, S, D)),
            "wqkv": _w((lambda *s: _rng.normal(s) * 0.1)(D, 3 * D)),
            "wo": _w((lambda *s: _rng.normal(s) * 0.05)(D, D)),
        }
    _A_in = _A_setup()

    def _B_setup():
        B, S, D, H = 1, 2048, 640, 32
        return {
            "x": _w((lambda *s: _rng.normal(s) * 0.05)(B, S, D)),
            "wqkv": _w((lambda *s: _rng.normal(s) * 0.1)(D, 3 * D)),
            "wo": _w((lambda *s: _rng.normal(s) * 0.05)(D, D)),
        }
    _B_in = _B_setup()

    return {
        "A_x": _A_in["x"],
        "A_wqkv": _A_in["wqkv"],
        "A_wo": _A_in["wo"],
        "B_x": _B_in["x"],
        "B_wqkv": _B_in["wqkv"],
        "B_wo": _B_in["wo"],
    }

def reference(A_x, A_wqkv, A_wo, B_x, B_wqkv, B_wo):
    def _A_ref(x, wqkv, wo):
        B, S, D = x.shape
        H = 32; Dh = D // H
        qkv = (lambda x, *d: x.transpose(*d))((x @ wqkv).reshape(B, S, 3, H, Dh), 2, 0, 3, 1, 4)
        q, k, v = qkv[0], qkv[1], qkv[2]
        phi = lambda t: jnp.where(t > 0, t + 1, jnp.exp(t)) + 1e-6
        pq, pk = phi(q), phi(k)
        kv = jnp.einsum("bhsd,bhse->bhde", pk, v)
        z = jnp.einsum("bhsd->bhd", pk)
        num = jnp.einsum("bhqd,bhde->bhqe", pq, kv)
        den = jnp.einsum("bhqd,bhd->bhq", pq, z)[..., None] + 1e-6
        o = num / den
        return (lambda x, *d: x.transpose(*d))(o, 0, 2, 1, 3).reshape(B, S, D) @ wo

    def _B_ref(x, wqkv, wo):
        B, S, D = x.shape
        H = 32
        Dh = D // H
        qkv = (lambda x, *d: x.transpose(*d))((x @ wqkv).reshape(B, S, 3, H, Dh), 2, 0, 3, 1, 4)
        q, k, v = qkv[0], qkv[1], qkv[2]
        scores = jnp.einsum("bhqd,bhkd->bhqk", q, k) * (Dh ** -0.5)
        p = _softmax(scores, axis=-1)
        o = jnp.einsum("bhqk,bhkd->bhqd", p, v)
        return (lambda x, *d: x.transpose(*d))(o, 0, 2, 1, 3).reshape(B, S, D) @ wo

    x = A_x
    x = x + _A_ref(_layernorm(x, axis=-1), A_wqkv, A_wo)
    x = x + _B_ref(_layernorm(x, axis=-1), B_wqkv, B_wo)
    x = x + _A_ref(_layernorm(x, axis=-1), A_wqkv, A_wo)
    x = x + _B_ref(_layernorm(x, axis=-1), B_wqkv, B_wo)
    return x
```

```python
import functools
import math

import jax
import jax.numpy as jnp
from jax import lax
from jax.experimental import pallas as pl
from jax.experimental.pallas import tpu as pltpu

_S = 2048
_D = 640
_H = 32
_DH = _D // _H
_T = 512
_NC = _S // _T
_CK = 128
_VR = 24
_NB = _D // 128
_LN_EPS = 1e-5
_QSCALE = (_DH ** -0.5) * math.log2(math.e)

_WIN = []
for _j in range(_NB):
    _lo = (128 * _j // _DH) * _DH
    _hi = -(-(128 * _j + 128) // _DH) * _DH
    _WIN.append((_lo // 16 * 16, min(_D, -(-_hi // 16) * 16)))
_WMAX = max(hi - lo for lo, hi in _WIN)

_F32 = jnp.float32
_BF16 = jnp.bfloat16


def _dot(a, b):
    return jnp.dot(a, b, preferred_element_type=_F32)


def _dot_nt(a, b):
    return lax.dot_general(a, b, (((1,), (1,)), ((), ())), preferred_element_type=_F32)


def _layernorm_t(x):
    mean = jnp.sum(x, axis=0, keepdims=True) * (1.0 / _D)
    d = x - mean
    var = jnp.sum(d * d, axis=0, keepdims=True) * (1.0 / _D)
    return (d * lax.rsqrt(var + _LN_EPS)).astype(_BF16)


def _phi(t):
    return jnp.where(t > 0, t + 1.0, jnp.exp(t)) + 1e-6


def _kernel(x_ref, aw_ref, awo_ref, bw_ref, bwo_ref, out_ref,
            xt_ref, awt_ref, awot_ref, bwt_ref, bwot_ref,
            qt_ref, k_ref, vt_ref, ot_ref, s_ref, kv_ref, lhs_ref):

    for j in range(3 * _NB):
        awt_ref[j * 128:(j + 1) * 128, :] = aw_ref[:, j * 128:(j + 1) * 128].T
        bwt_ref[j * 128:(j + 1) * 128, :] = bw_ref[:, j * 128:(j + 1) * 128].T
    for j in range(_NB):
        awot_ref[j * 128:(j + 1) * 128, :] = awo_ref[:, j * 128:(j + 1) * 128].T
        bwot_ref[j * 128:(j + 1) * 128, :] = bwo_ref[:, j * 128:(j + 1) * 128].T
    tail = jnp.where(lax.broadcasted_iota(jnp.int32, (8, _T), 0) == _DH - 16, 1.0, 0.0).astype(_F32)

    def init_vt(i, carry):
        vt_ref[i // _H, i % _H, 16:24, :] = tail
        return carry
    lax.fori_loop(0, _NC * _H, init_vt, 0)

    def lin_front(c, xt):
        xn = _layernorm_t(xt)
        pq = _phi(_dot(awt_ref[0:_D, :], xn)).astype(_BF16)
        for j in range(_NB):
            qt_ref[c, j] = pq[j * 128:(j + 1) * 128, :]
        pk = _phi(_dot(awt_ref[_D:2 * _D, :], xn)).astype(_BF16)
        v = _dot(awt_ref[2 * _D:3 * _D, :], xn).astype(_BF16)
        ones = jnp.ones((16, _T), _BF16)
        for j, (lo, hi) in enumerate(_WIN):
            lhs = jnp.concatenate([ones, v[lo:hi, :]], axis=0)
            kv_ref[j, 0:16 + hi - lo, :] += _dot_nt(lhs, pk[j * 128:(j + 1) * 128, :])

    def lin_mid():
        for j, (lo, hi) in enumerate(_WIN):
            n = hi - lo
            e = lax.broadcasted_iota(jnp.int32, (n, 128), 0) + lo
            d = lax.broadcasted_iota(jnp.int32, (n, 128), 1) + 128 * j
            same = None
            for h in range(lo // _DH, -(-hi // _DH)):
                a, b = h * _DH, (h + 1) * _DH
                m = (e >= a) & (e < b) & (d >= a) & (d < b)
                same = m if same is None else (same | m)
            z = jnp.broadcast_to(kv_ref[j, 0:1, :], (n, 128))
            lhs_ref[j, 0:n, :] = jnp.where(same, kv_ref[j, 16:16 + n, :], 0.0).astype(_BF16)
            lhs_ref[j, n:2 * n, :] = jnp.where(same, z, 0.0).astype(_BF16)

    def lin_back(c):
        parts = []
        for j, (lo, hi) in enumerate(_WIN):
            parts.append(_dot(lhs_ref[j, 0:2 * (hi - lo), :], qt_ref[c, j]))
        edges = sorted({e for w in _WIN for e in w})
        outs = []
        for a, b in zip(edges[:-1], edges[1:]):
            num = den = None
            for j, (lo, hi) in enumerate(_WIN):
                if lo <= a and b <= hi:
                    n = hi - lo
                    pn = parts[j][a - lo:b - lo, :]
                    pd = parts[j][n + a - lo:n + b - lo, :]
                    num = pn if num is None else num + pn
                    den = pd if den is None else den + pd
            outs.append((num / (den + 1e-6)).astype(_BF16))
        o = jnp.concatenate(outs, axis=0)
        return xt_ref[c] + _dot(awot_ref[...], o)

    def mha_front(c, xt):
        xn = _layernorm_t(xt)
        q = (_dot(bwt_ref[0:_D, :], xn) * _QSCALE).astype(_BF16)
        for j in range(_NB):
            qt_ref[c, j] = q[j * 128:(j + 1) * 128, :]
        for j in range(_NB - 1):
            qt_ref[c, _NB + j, 0:64, :] = q[(j + 1) * 128:(j + 1) * 128 + 64, :]
            qt_ref[c, _NB + j, 64:128, :] = q[j * 128 + 64:(j + 1) * 128, :]
        kt = _dot(bwt_ref[_D:2 * _D, :], xn).astype(_BF16)
        kb = [pltpu.bitcast(kt[j * 128:(j + 1) * 128, :].T, jnp.int32) for j in range(_NB)]
        low = lax.broadcasted_iota(jnp.int32, (_T // 2, 128), 1) < 64
        for j in range(_NB):
            k_ref[j, c] = pltpu.bitcast(kb[j], _BF16)
        for j in range(_NB - 1):
            k_ref[_NB + j, c] = pltpu.bitcast(jnp.where(low, kb[j + 1], kb[j]), _BF16)
        v = _dot(bwt_ref[2 * _D:3 * _D, :], xn)
        for h in range(_H):
            vt_ref[c, h, 0:_DH, :] = v[h * _DH:(h + 1) * _DH, :]

    def mha_back(c):
        o = jnp.concatenate([ot_ref[c, h, 0:_DH, :] for h in range(_H)], axis=0).astype(_BF16)
        return xt_ref[c] + _dot(bwot_ref[...], o)

    n_steps = _H * _NC

    def head_q(i):
        h = i // _NC
        c = i % _NC
        start = h * _DH
        off = start % 128
        jb = start // 128 + jnp.where(off > 128 - _DH, _NB, 0)
        q = pltpu.bitcast(qt_ref[c, jb], jnp.int32)
        r = lax.broadcasted_iota(jnp.int32, (64, _T), 0)
        keep = ((r - off // 2) & 63) < _DH // 2
        return jb, pltpu.bitcast(jnp.where(keep, q, 0), _BF16)

    def scores(jb, qm, t):
        cc, r0 = divmod(t * _CK, _T)
        s = _dot(k_ref[jb, cc, r0:r0 + _CK, :], qm)
        s_ref[t * _CK:(t + 1) * _CK, :] = s
        return jnp.max(s.reshape(_CK // 8, 8, _T), axis=0)

    def weighted(h, sc, m, t):
        cc, r0 = divmod(t * _CK, _T)
        return _dot(vt_ref[cc, h, :, r0:r0 + _CK], jnp.exp2(sc - m))

    def finish(i, acc):
        ot_ref[i % _NC, i // _NC] = acc / acc[_DH:_DH + 1, :]

    def attention():
        jb, qm = head_q(0)
        mx = None
        for t in range(_S // _CK):
            cm = scores(jb, qm, t)
            mx = cm if mx is None else jnp.maximum(mx, cm)

        def step(i, m):
            jb, qm = head_q(i + 1)
            h = i // _NC
            mx = acc = None
            for t in range(_S // _CK):
                sc = s_ref[t * _CK:(t + 1) * _CK, :]
                cm = scores(jb, qm, t)
                mx = cm if mx is None else jnp.maximum(mx, cm)
                ov = weighted(h, sc, m, t)
                acc = ov if acc is None else acc + ov
            finish(i, acc)
            return jnp.max(mx, axis=0, keepdims=True)

        m = lax.fori_loop(0, n_steps - 1, step, jnp.max(mx, axis=0, keepdims=True))
        acc = None
        for t in range(_S // _CK):
            ov = weighted(_H - 1, s_ref[t * _CK:(t + 1) * _CK, :], m, t)
            acc = ov if acc is None else acc + ov
        finish(n_steps - 1, acc)

    def rows(c):
        return pl.ds(pl.multiple_of(c * _T, _T), _T)

    def for_chunks(body):
        def wrapped(c, carry):
            body(c)
            return carry
        lax.fori_loop(0, _NC, wrapped, 0)

    def first(c):
        xt = x_ref[rows(c), :].T.astype(_F32)
        xt_ref[c] = xt
        lin_front(c, xt)

    def lin_to_mha(c):
        xt = lin_back(c)
        xt_ref[c] = xt
        mha_front(c, xt)

    def mha_to_lin(c):
        xt = mha_back(c)
        xt_ref[c] = xt
        lin_front(c, xt)

    def last(c):
        out_ref[rows(c), :] = mha_back(c).astype(_BF16).T

    kv_ref[...] = jnp.zeros(kv_ref.shape, _F32)
    for_chunks(first)
    lin_mid()
    for_chunks(lin_to_mha)
    attention()
    kv_ref[...] = jnp.zeros(kv_ref.shape, _F32)
    for_chunks(mha_to_lin)
    lin_mid()
    for_chunks(lin_to_mha)
    attention()
    for_chunks(last)


@jax.jit
def pallas_interleave_layers__linear_attn_block__mha_block__prompt_kernel(
    A_x: jax.Array,
    A_wqkv: jax.Array,
    A_wo: jax.Array,
    B_x: jax.Array,
    B_wqkv: jax.Array,
    B_wo: jax.Array,
):
    del B_x
    out = pl.pallas_call(
        _kernel,
        out_shape=jax.ShapeDtypeStruct((_S, _D), _BF16),
        scratch_shapes=[
            pltpu.VMEM((_NC, _D, _T), _F32),
            pltpu.VMEM((3 * _D, _D), _BF16),
            pltpu.VMEM((_D, _D), _BF16),
            pltpu.VMEM((3 * _D, _D), _BF16),
            pltpu.VMEM((_D, _D), _BF16),
            pltpu.VMEM((_NC, 2 * _NB - 1, 128, _T), _BF16),
            pltpu.VMEM((2 * _NB - 1, _NC, _T, 128), _BF16),
            pltpu.VMEM((_NC, _H, _VR, _T), _F32),
            pltpu.VMEM((_NC, _H, _VR, _T), _F32),
            pltpu.VMEM((_S, _T), _F32),
            pltpu.VMEM((_NB, 16 + _WMAX, 128), _F32),
            pltpu.VMEM((_NB, 2 * _WMAX, 128), _BF16),
        ],
        compiler_params=pltpu.CompilerParams(vmem_limit_bytes=100 * 1024 * 1024),
    )(A_x.reshape(_S, _D), A_wqkv, A_wo, B_wqkv, B_wo)
    return out.reshape(A_x.shape)
```

```python
import math

import jax
import jax.numpy as jnp
from jax import lax
from jax.experimental import pallas as pl
from jax.experimental.pallas import tpu as pltpu

_S = 2048
_D = 640
_H = 32
_DH = _D // _H
_T = 512
_NC = _S // _T
_CK = 128
_NT = _S // _CK
_VR = 24
_NB = _D // 128
_LN_EPS = 1e-5
_QSCALE = (_DH ** -0.5) * math.log2(math.e)

_WIN = []
for _j in range(_NB):
    _lo = (128 * _j // _DH) * _DH
    _hi = -(-(128 * _j + 128) // _DH) * _DH
    _WIN.append((_lo // 16 * 16, min(_D, -(-_hi // 16) * 16)))

_F32 = jnp.float32
_BF16 = jnp.bfloat16


_I32 = jnp.int32


def _pack(x):
    return pltpu.bitcast(x.astype(_BF16), _I32)


def _operand(x):
    return pltpu.bitcast(x, _BF16) if x.dtype == _I32 else x


def _dot(a, b):
    return jnp.dot(_operand(a), _operand(b), preferred_element_type=_F32)


def _dot_nt(a, b):
    return lax.dot_general(a, b, (((1,), (1,)), ((), ())), preferred_element_type=_F32)


def _blocks(x):
    return [x[r:r + 128, :].astype(_BF16) for r in range(0, x.shape[0], 128)]


def _layernorm_t(x):
    mean = jnp.sum(x, axis=0, keepdims=True) * (1.0 / _D)
    d = x - mean
    var = jnp.sum(d * d, axis=0, keepdims=True) * (1.0 / _D)
    return d * lax.rsqrt(var + _LN_EPS)


def _phi(t):
    return jnp.where(t > 0, t + 1.0, jnp.exp(t)) + 1e-6


def _windows(v):
    ones = jnp.ones((16, v.shape[1]), _F32)
    return [jnp.concatenate([ones, v[lo:hi, :]], axis=0).astype(_BF16) for lo, hi in _WIN]


def _iota(shape, axis):
    return lax.broadcasted_iota(_I32, shape, axis)


def _kernel(x_hbm, aw_hbm, awo_hbm, bw_hbm, bwo_hbm, out_hbm,
            x_ref, aw_ref, awo_ref, bw_ref, bwo_ref, out_ref,
            xt_ref, awt_ref, awot_ref, bwt_ref, bwot_ref,
            qt_ref, k_ref, vt_ref, ot_ref, s_ref, m_ref, in_sem, out_sem):

    def rows(c):
        return pl.ds(c * _T, _T)

    def cols(i):
        return pl.ds(i * _D, _D)

    x_cp = [pltpu.make_async_copy(x_hbm.at[rows(c)], x_ref.at[rows(c)], in_sem.at[c])
            for c in range(_NC)]
    aw_cp = [pltpu.make_async_copy(aw_hbm.at[:, cols(i)], aw_ref.at[:, cols(i)], in_sem.at[_NC + i])
             for i in range(3)]
    awo_cp = pltpu.make_async_copy(awo_hbm, awo_ref, in_sem.at[_NC + 3])
    bw_cp = pltpu.make_async_copy(bw_hbm, bw_ref, in_sem.at[_NC + 4])
    bwo_cp = pltpu.make_async_copy(bwo_hbm, bwo_ref, in_sem.at[_NC + 5])
    out_cp = [pltpu.make_async_copy(out_ref.at[rows(c)], out_hbm.at[rows(c)], out_sem.at[c])
              for c in range(_NC)]

    def head_block(h):
        start = h * _DH
        off = start & 127
        return (start >> 7) + jnp.where(off > 128 - _DH, _NB, 0), off >> 1

    def masked_q(c, jb, off2):
        keep = ((_iota((64, _T), 0) - off2) & 63) < _DH // 2
        return jnp.where(keep, qt_ref[c, jb], 0)

    def scores(c, jb, qm, t):
        cc, r0 = divmod(t * _CK, _T)
        s = _dot(k_ref[jb, cc, r0 // 2:(r0 + _CK) // 2, :], qm)
        s_ref[c, t * _CK:(t + 1) * _CK, :] = s
        return jnp.max(s.reshape(_CK // 8, 8, _T), axis=0)

    def weighted(h, sc, m, t):
        cc, r0 = divmod(t * _CK, _T)
        return _dot(vt_ref[cc, h, :, r0:r0 + _CK], jnp.exp2(sc - m))

    def normalise(acc):
        return acc / acc[_DH:_DH + 1, :]

    def first_head():
        def body(c, carry):
            jb, off2 = head_block(0)
            qm = masked_q(c, jb, off2)
            mx = None
            for t in range(_NT):
                cm = scores(c, jb, qm, t)
                mx = cm if mx is None else jnp.maximum(mx, cm)
            m_ref[c] = jnp.max(mx, axis=0, keepdims=True)
            return carry
        lax.fori_loop(0, _NC, body, 0)

    def middle_heads():
        def body(h, carry):
            jb, off2 = head_block(h + 1)
            for c in range(_NC):
                qm = masked_q(c, jb, off2)
                m = m_ref[c]
                mx = acc = None
                for t in range(_NT):
                    sc = s_ref[c, t * _CK:(t + 1) * _CK, :]
                    cm = scores(c, jb, qm, t)
                    mx = cm if mx is None else jnp.maximum(mx, cm)
                    ov = weighted(h, sc, m, t)
                    acc = ov if acc is None else acc + ov
                ot_ref[c, h] = normalise(acc)
                m_ref[c] = jnp.max(mx, axis=0, keepdims=True)
            return carry
        lax.fori_loop(0, _H - 1, body, 0)

    pending = []

    class Lazy:
        def __init__(self, pieces):
            self.pieces = list(pieces)
            self.values = []
            pending.append(self)

        def step(self):
            self.values.append(self.pieces[len(self.values)]())
            if len(self.values) == len(self.pieces):
                pending.remove(self)

        def get(self):
            while len(self.values) < len(self.pieces):
                self.step()
            return self.values

        def lanes(self):
            return jnp.concatenate(self.get(), axis=1).astype(_BF16)

    def fill():
        for lazy in list(pending):
            lazy.step()

    def project(w_ref, lo, hi, rhs, rows_per_piece=128):
        outs = []
        for r in range(lo, hi, rows_per_piece):
            outs.append(_dot(w_ref[r // 2:(r + rows_per_piece) // 2, :], rhs))
            fill()
        return jnp.concatenate(outs, axis=0)

    def lane_pieces(fn):
        return Lazy([lambda i=i: fn(slice(i * 128, (i + 1) * 128)) for i in range(_T // 128)])

    def transpose_weight(src, dst, lo, hi):
        def piece(j):
            dst[j * 64:(j + 1) * 64, :] = _pack(src[:, j * 128:(j + 1) * 128].astype(_F32).T)
        return Lazy([lambda j=j: piece(j) for j in range(lo, hi)])

    def residual_ln(c, delta):
        xt = xt_ref[c] + delta
        xt_ref[c] = xt
        return lane_pieces(lambda ls: _layernorm_t(xt[:, ls]))

    def last_head(c):
        def piece(t0):
            acc = None
            for t in range(t0, t0 + 4):
                ov = weighted(_H - 1, s_ref[c, t * _CK:(t + 1) * _CK, :], m_ref[c], t)
                acc = ov if acc is None else acc + ov
            return acc
        return Lazy([lambda t0=t0: piece(t0) for t0 in range(0, _NT, 4)])

    def mha_out(c, last):
        parts = last.get()
        acc = parts[0]
        for p in parts[1:]:
            acc = acc + p
        heads = [ot_ref[c, h, 0:_DH, :] for h in range(_H - 1)] + [normalise(acc)[0:_DH, :]]
        return project(bwot_ref, 0, _D, jnp.concatenate(heads, axis=0).astype(_BF16))

    def lin_kv(xn):
        pk = _blocks(_phi(project(awt_ref, _D, 2 * _D, xn)))
        v = _windows(project(awt_ref, 2 * _D, 3 * _D, xn))
        return pk, v

    def lin_q(xn, lo=0, hi=_D):
        return _blocks(_phi(project(awt_ref, lo, hi, xn)))

    def lin_state(state, pk, v):
        parts = [_dot_nt(v[j], pk[j]) for j in range(_NB)]
        return parts if state is None else [a + b for a, b in zip(state, parts)]

    def lin_front(state, xn, last=False):
        pk, v = lin_kv(xn)
        if not last:
            pq = lin_q(xn)
            return lin_state(state, pk, v), pq
        q_lo = lin_q(xn, 0, 256)
        ops = lin_operands(lin_state(state, pk, v))
        return ops, q_lo + lin_q(xn, 256, _D)

    def lin_operands(state):
        def head_of(i):
            return (i * 3277) >> 16

        def piece(j):
            lo, hi = _WIN[j]
            n = hi - lo
            hd = head_of(_iota((1, 128), 1) + 128 * j)
            kv = jnp.where(head_of(_iota((n, 128), 0) + lo) == hd, state[j][16:16 + n, :], 0.0)
            z = jnp.where(_iota((_H, 128), 0) == hd, state[j][0:1, :], 0.0)
            return _pack(jnp.concatenate([z, kv], axis=0))
        return Lazy([lambda j=j: piece(j) for j in range(_NB)])

    def lin_read(ops, pq):
        parts = [_dot(ops[j], pq[j]) for j in range(_NB)]

        def piece(ls):
            den = parts[0][0:_H, ls]
            for j in range(1, _NB):
                den = den + parts[j][0:_H, ls]
            inv = 1.0 / (den + 1e-6)
            sub = _iota((8, 128), 0)
            groups = []
            for a in range(0, _D, 8):
                num = None
                for j, (lo, hi) in enumerate(_WIN):
                    if lo <= a < hi:
                        p = parts[j][_H + a - lo:_H + a - lo + 8, ls]
                        num = p if num is None else num + p
                h = a // _DH
                scale = jnp.broadcast_to(inv[h:h + 1, :], (8, 128))
                split = (h + 1) * _DH - a
                if split < 8:
                    scale = jnp.where(sub < split, scale, jnp.broadcast_to(inv[h + 1:h + 2, :], (8, 128)))
                groups.append(num * scale)
            return jnp.concatenate(groups, axis=0)
        return lane_pieces(piece)

    def lin_out(c, o):
        return residual_ln(c, project(awot_ref, 0, _D, o.lanes()))

    def mha_in(c, xn):
        xn = xn.lanes()
        kt = project(bwt_ref, _D, 2 * _D, xn)
        kb = []

        def k_piece(j):
            kb.append(_pack(kt[j * 128:(j + 1) * 128, :].T))
            k_ref[j, c] = kb[j]
            if j > 0:
                low = _iota((_T // 2, 128), 1) < 64
                k_ref[_NB + j - 1, c] = jnp.where(low, kb[j], kb[j - 1])
        Lazy([lambda j=j: k_piece(j) for j in range(_NB)])

        v = project(bwt_ref, 2 * _D, 3 * _D, xn)

        def v_piece(h0):
            tail = jnp.where(_iota((_VR - _DH, _T), 0) == 0, 1.0, 0.0).astype(_F32)
            for h in range(h0, h0 + 8):
                vt_ref[c, h] = jnp.concatenate([v[h * _DH:(h + 1) * _DH, :], tail], axis=0)
        Lazy([lambda h0=h0: v_piece(h0) for h0 in range(0, _H, 8)])

        q = _pack(project(bwt_ref, 0, _D, xn) * _QSCALE)
        for j in range(_NB):
            qt_ref[c, j] = q[j * 64:(j + 1) * 64, :]
        for j in range(_NB - 1):
            qt_ref[c, _NB + j, 0:32, :] = q[(j + 1) * 64:(j + 1) * 64 + 32, :]
            qt_ref[c, _NB + j, 32:64, :] = q[j * 64 + 32:(j + 1) * 64, :]

    def lin_back_mha_front(ops, pq):
        ops = ops.get()
        o0 = lin_read(ops, pq[0])
        o1 = lin_read(ops, pq[1])
        o0.get()
        o2 = lin_read(ops, pq[2])
        xn0 = lin_out(0, o0)
        o3 = lin_read(ops, pq[3])
        xn1 = lin_out(1, o1)
        mha_in(0, xn0)
        xn2 = lin_out(2, o2)
        mha_in(1, xn1)
        xn3 = lin_out(3, o3)
        mha_in(2, xn2)
        mha_in(3, xn3)
        while pending:
            fill()

    x_cp[0].start()
    aw_cp[1].start()
    aw_cp[2].start()
    aw_cp[0].start()
    for c in range(1, _NC):
        x_cp[c].start()
    awo_cp.start()
    bw_cp.start()
    bwo_cp.start()

    def load_chunk(c):
        x_cp[c].wait()

        def piece(ls):
            xt = x_ref[c * _T + ls.start:c * _T + ls.stop, :].astype(_F32).T
            xt_ref[c, :, ls] = xt
            return _layernorm_t(xt)
        return lane_pieces(piece)

    xn = load_chunk(0).lanes()
    aw_cp[1].wait()
    transpose_weight(aw_ref, awt_ref, _NB, 2 * _NB).get()
    aw_cp[2].wait()
    wv = transpose_weight(aw_ref, awt_ref, 2 * _NB, 3 * _NB)
    pk = _blocks(_phi(project(awt_ref, _D, 2 * _D, xn)))
    wv.get()
    aw_cp[0].wait()
    wq = transpose_weight(aw_ref, awt_ref, 0, _NB)
    v = _windows(project(awt_ref, 2 * _D, 3 * _D, xn))
    wq.get()
    xn_next = load_chunk(1)
    pq = [lin_q(xn)]
    state = lin_state(None, pk, v)
    later = [(awo_cp, awo_ref, awot_ref, _NB), (bw_cp, bw_ref, bwt_ref, 3 * _NB),
             (bwo_cp, bwo_ref, bwot_ref, _NB)]
    for c in range(1, _NC):
        xn = xn_next.lanes()
        if c + 1 < _NC:
            xn_next = load_chunk(c + 1)
        cp, src, dst, n = later[c - 1]
        cp.wait()
        transpose_weight(src, dst, 0, n)
        state, q = lin_front(state, xn, last=c + 1 == _NC)
        pq.append(q)
    lin_back_mha_front(state, pq)

    first_head()
    middle_heads()

    tails = [last_head(0)]
    tails[0].get()
    tails.append(last_head(1))
    xn0 = residual_ln(0, mha_out(0, tails[0]))
    tails.append(last_head(2))
    xn1 = residual_ln(1, mha_out(1, tails[1]))
    tails.append(last_head(3))
    state, q = lin_front(None, xn0.lanes())
    pq = [q]
    xn2 = residual_ln(2, mha_out(2, tails[2]))
    state, q = lin_front(state, xn1.lanes())
    pq.append(q)
    xn3 = residual_ln(3, mha_out(3, tails[3]))
    state, q = lin_front(state, xn2.lanes())
    pq.append(q)
    state, q = lin_front(state, xn3.lanes(), last=True)
    pq.append(q)
    lin_back_mha_front(state, pq)

    first_head()
    middle_heads()

    def store_chunk(c, xt):
        def piece(ls):
            out_ref[c * _T + ls.start:c * _T + ls.stop, :] = xt[:, ls].T.astype(_BF16)
            if ls.stop == _T:
                out_cp[c].start()
        return lane_pieces(piece)

    tails = [last_head(0)]
    tails[0].get()
    for c in range(_NC):
        if c + 1 < _NC:
            tails.append(last_head(c + 1))
        store_chunk(c, xt_ref[c] + mha_out(c, tails[c]))
    while pending:
        fill()
    for c in range(_NC):
        out_cp[c].wait()


@jax.jit
def pallas_interleave_layers__linear_attn_block__mha_block__prompt_kernel(
    A_x: jax.Array,
    A_wqkv: jax.Array,
    A_wo: jax.Array,
    B_x: jax.Array,
    B_wqkv: jax.Array,
    B_wo: jax.Array,
):
    del B_x
    any_spec = pl.BlockSpec(memory_space=pl.ANY)
    out = pl.pallas_call(
        _kernel,
        out_shape=jax.ShapeDtypeStruct((_S, _D), _BF16),
        in_specs=[any_spec] * 5,
        out_specs=any_spec,
        scratch_shapes=[
            pltpu.VMEM((_S, _D), _BF16),
            pltpu.VMEM((_D, 3 * _D), _BF16),
            pltpu.VMEM((_D, _D), _BF16),
            pltpu.VMEM((_D, 3 * _D), _BF16),
            pltpu.VMEM((_D, _D), _BF16),
            pltpu.VMEM((_S, _D), _BF16),
            pltpu.VMEM((_NC, _D, _T), _F32),
            pltpu.VMEM((3 * _D // 2, _D), _I32),
            pltpu.VMEM((_D // 2, _D), _I32),
            pltpu.VMEM((3 * _D // 2, _D), _I32),
            pltpu.VMEM((_D // 2, _D), _I32),
            pltpu.VMEM((_NC, 2 * _NB - 1, 64, _T), _I32),
            pltpu.VMEM((2 * _NB - 1, _NC, _T // 2, 128), _I32),
            pltpu.VMEM((_NC, _H, _VR, _T), _F32),
            pltpu.VMEM((_NC, _H, _VR, _T), _F32),
            pltpu.VMEM((_NC, _S, _T), _F32),
            pltpu.VMEM((_NC, 1, _T), _F32),
            pltpu.SemaphoreType.DMA((_NC + 6,)),
            pltpu.SemaphoreType.DMA((_NC,)),
        ],
        compiler_params=pltpu.CompilerParams(vmem_limit_bytes=110 * 1024 * 1024),
    )(A_x.reshape(_S, _D), A_wqkv, A_wo, B_wqkv, B_wo)
    return out.reshape(A_x.shape)
```

```python
import math

import jax
import jax.numpy as jnp
from jax import lax
from jax.experimental import pallas as pl
from jax.experimental.pallas import tpu as pltpu

_S = 2048
_D = 640
_H = 32
_DH = _D // _H
_T = 512
_NC = _S // _T
_CK = 128
_NT = _S // _CK
_VR = 24
_NB = _D // 128
_LN_EPS = 1e-5
_QSCALE = (_DH ** -0.5) * math.log2(math.e)

_WIN = []
for _j in range(_NB):
    _lo = (128 * _j // _DH) * _DH
    _hi = -(-(128 * _j + 128) // _DH) * _DH
    _WIN.append((_lo // 16 * 16, min(_D, -(-_hi // 16) * 16)))

_F32 = jnp.float32
_BF16 = jnp.bfloat16


_I32 = jnp.int32


def _pack(x):
    return pltpu.bitcast(x.astype(_BF16), _I32)


def _operand(x):
    return pltpu.bitcast(x, _BF16) if x.dtype == _I32 else x


def _dot(a, b):
    return jnp.dot(_operand(a), _operand(b), preferred_element_type=_F32)


def _dot_nt(a, b):
    return lax.dot_general(a, b, (((1,), (1,)), ((), ())), preferred_element_type=_F32)


def _blocks(x):
    return [x[r:r + 128, :].astype(_BF16) for r in range(0, x.shape[0], 128)]


def _layernorm_t(x):
    mean = jnp.sum(x, axis=0, keepdims=True) * (1.0 / _D)
    d = x - mean
    var = jnp.sum(d * d, axis=0, keepdims=True) * (1.0 / _D)
    return d * lax.rsqrt(var + _LN_EPS)


def _phi(t):
    return jnp.where(t > 0, t + 1.0, jnp.exp(t)) + 1e-6


def _windows(v):
    ones = jnp.ones((16, v.shape[1]), _F32)
    return [jnp.concatenate([ones, v[lo:hi, :]], axis=0).astype(_BF16) for lo, hi in _WIN]


def _iota(shape, axis):
    return lax.broadcasted_iota(_I32, shape, axis)


def _kernel(x_hbm, aw_hbm, awo_hbm, bw_hbm, bwo_hbm, out_hbm,
            x_ref, aw_ref, awo_ref, bw_ref, bwo_ref, out_ref,
            xt_ref, awt_ref, awot_ref, bwt_ref, bwot_ref,
            qt_ref, k_ref, vt_ref, ot_ref, on_ref, s_ref, m_ref, qm_ref, in_sem, out_sem):

    def rows(c):
        return pl.ds(c * _T, _T)

    def cols(i):
        return pl.ds(i * _D, _D)

    x_cp = [pltpu.make_async_copy(x_hbm.at[rows(c)], x_ref.at[rows(c)], in_sem.at[c])
            for c in range(_NC)]
    aw_cp = [pltpu.make_async_copy(aw_hbm.at[:, cols(i)], aw_ref.at[:, cols(i)], in_sem.at[_NC + i])
             for i in range(3)]
    awo_cp = pltpu.make_async_copy(awo_hbm, awo_ref, in_sem.at[_NC + 3])
    bw_cp = pltpu.make_async_copy(bw_hbm, bw_ref, in_sem.at[_NC + 4])
    bwo_cp = pltpu.make_async_copy(bwo_hbm, bwo_ref, in_sem.at[_NC + 5])
    out_cp = [pltpu.make_async_copy(out_ref.at[rows(c)], out_hbm.at[rows(c)], out_sem.at[c])
              for c in range(_NC)]

    def head_block(h):
        start = h * _DH
        off = start & 127
        return (start >> 7) + jnp.where(off > 128 - _DH, _NB, 0), off >> 1

    def masked_q(c, jb, off2):
        keep = ((_iota((64, _T), 0) - off2) & 63) < _DH // 2
        return jnp.where(keep, qt_ref[c, jb], 0)

    def scores(c, jb, qm, t):
        cc, r0 = divmod(t * _CK, _T)
        s = _dot(k_ref[jb, cc, r0 // 2:(r0 + _CK) // 2, :], qm)
        s_ref[c, t * _CK:(t + 1) * _CK, :] = s
        return jnp.max(s.reshape(_CK // 8, 8, _T), axis=0)

    def values(h, t):
        cc, r0 = divmod(t * _CK, _T)
        return vt_ref[cc, h, :, r0:r0 + _CK]

    def normalise(acc):
        return acc * (1.0 / acc[_DH:_DH + 1, :])

    def finish(h, c, acc, mx):
        ot_ref[c, h + 1] = acc
        m_ref[c] = jnp.max(mx, axis=0, keepdims=True)

    def stage_q(h):
        jb, off2 = head_block(h)
        qm_ref[...] = masked_q(0, jb, off2)
        return jb, off2

    def first_head():
        def body(_, carry):
            jb, off2 = head_block(0)
            for c in range(_NC):
                qm = masked_q(c, jb, off2)
                mx = None
                for t in range(_NT):
                    cm = scores(c, jb, qm, t)
                    mx = cm if mx is None else jnp.maximum(mx, cm)
                m_ref[c] = jnp.max(mx, axis=0, keepdims=True)
            return carry
        lax.fori_loop(0, 1, body, 0)

    def middle_heads():
        def body(h, carry):
            jb, off2 = carry
            qm = qm_ref[...]

            def probs(n):
                c, t = divmod(n, _NT)
                return jnp.exp2(s_ref[c, t * _CK:(t + 1) * _CK, :] - m_ref[c])

            for c in range(_NC):
                on_ref[c, h] = normalise(ot_ref[c, h])
            p_next = probs(0)
            done = None
            for n in range(_NC * _NT):
                c, t = divmod(n, _NT)
                p = p_next
                if n + 1 < _NC * _NT:
                    p_next = probs(n + 1)
                cm = scores(c, jb, qm, t)
                mx = cm if t == 0 else jnp.maximum(mx, cm)
                ov = _dot(values(h, t), p)
                acc = ov if t == 0 else acc + ov
                if t == 1 and done is not None:
                    finish(h, *done)
                if t == _NT - 4:
                    if c + 1 < _NC:
                        qm_next = masked_q(c + 1, jb, off2)
                    else:
                        carry = stage_q(jnp.minimum(h + 2, _H - 1))
                if t == _NT - 1:
                    done = (c, acc, mx)
                    qm = qm_next
            finish(h, *done)
            return carry
        lax.fori_loop(0, _H - 1, body, stage_q(1))

    pending = []

    class Lazy:
        def __init__(self, pieces):
            self.pieces = list(pieces)
            self.values = []
            pending.append(self)

        def step(self):
            self.values.append(self.pieces[len(self.values)]())
            if len(self.values) == len(self.pieces):
                pending.remove(self)

        def get(self):
            while len(self.values) < len(self.pieces):
                self.step()
            return self.values

        def lanes(self):
            return jnp.concatenate(self.get(), axis=1).astype(_BF16)

    def fill():
        for lazy in list(pending):
            lazy.step()

    def project(w_ref, lo, hi, rhs, rows_per_piece=128):
        outs = []
        for r in range(lo, hi, rows_per_piece):
            outs.append(_dot(w_ref[r // 2:(r + rows_per_piece) // 2, :], rhs))
            fill()
        return jnp.concatenate(outs, axis=0)

    def lane_pieces(fn):
        return Lazy([lambda i=i: fn(slice(i * 128, (i + 1) * 128)) for i in range(_T // 128)])

    def transpose_weight(src, dst, lo, hi):
        def piece(j):
            dst[j * 64:(j + 1) * 64, :] = _pack(src[:, j * 128:(j + 1) * 128].astype(_F32).T)
        return Lazy([lambda j=j: piece(j) for j in range(lo, hi)])

    def residual_ln(c, delta):
        xt = xt_ref[c] + delta
        xt_ref[c] = xt
        return lane_pieces(lambda ls: _layernorm_t(xt[:, ls]))

    def last_head(c):
        def piece(t0):
            acc = None
            for t in range(t0, t0 + 4):
                ov = _dot(values(_H - 1, t), jnp.exp2(s_ref[c, t * _CK:(t + 1) * _CK, :] - m_ref[c]))
                acc = ov if acc is None else acc + ov
            return acc
        return Lazy([lambda t0=t0: piece(t0) for t0 in range(0, _NT, 4)])

    def mha_out(c, tail):
        parts = tail.get()
        acc = parts[0]
        for p in parts[1:]:
            acc = acc + p
        heads = [on_ref[c, h + 1, 0:_DH, :] for h in range(_H - 2)]
        heads += [normalise(ot_ref[c, _H - 1])[0:_DH, :], normalise(acc)[0:_DH, :]]
        o = jnp.concatenate(heads, axis=0)
        return project(bwot_ref, 0, _D, o.astype(_BF16))

    def lin_kv(xn):
        pk = _blocks(_phi(project(awt_ref, _D, 2 * _D, xn)))
        v = _windows(project(awt_ref, 2 * _D, 3 * _D, xn))
        return pk, v

    def lin_q(xn, lo=0, hi=_D):
        return _blocks(_phi(project(awt_ref, lo, hi, xn)))

    def lin_state(state, pk, v):
        parts = [_dot_nt(v[j], pk[j]) for j in range(_NB)]
        return parts if state is None else [a + b for a, b in zip(state, parts)]

    def lin_front(state, xn, last=False):
        pk, v = lin_kv(xn)
        if not last:
            pq = lin_q(xn)
            return lin_state(state, pk, v), pq
        q_lo = lin_q(xn, 0, 256)
        ops = lin_operands(lin_state(state, pk, v))
        return ops, q_lo + lin_q(xn, 256, _D)

    def lin_operands(state):
        def head_of(i):
            return (i * 3277) >> 16

        def piece(j):
            lo, hi = _WIN[j]
            n = hi - lo
            hd = head_of(_iota((1, 128), 1) + 128 * j)
            kv = jnp.where(head_of(_iota((n, 128), 0) + lo) == hd, state[j][16:16 + n, :], 0.0)
            z = jnp.where(_iota((_H, 128), 0) == hd, state[j][0:1, :], 0.0)
            return _pack(jnp.concatenate([z, kv], axis=0))
        return Lazy([lambda j=j: piece(j) for j in range(_NB)])

    def lin_read(ops, pq):
        parts = [_dot(ops[j], pq[j]) for j in range(_NB)]

        def piece(ls):
            den = parts[0][0:_H, ls]
            for j in range(1, _NB):
                den = den + parts[j][0:_H, ls]
            inv = 1.0 / (den + 1e-6)
            sub = _iota((8, 128), 0)
            groups = []
            for a in range(0, _D, 8):
                num = None
                for j, (lo, hi) in enumerate(_WIN):
                    if lo <= a < hi:
                        p = parts[j][_H + a - lo:_H + a - lo + 8, ls]
                        num = p if num is None else num + p
                h = a // _DH
                scale = jnp.broadcast_to(inv[h:h + 1, :], (8, 128))
                split = (h + 1) * _DH - a
                if split < 8:
                    scale = jnp.where(sub < split, scale, jnp.broadcast_to(inv[h + 1:h + 2, :], (8, 128)))
                groups.append(num * scale)
            return jnp.concatenate(groups, axis=0)
        return lane_pieces(piece)

    def lin_out(c, o):
        return residual_ln(c, project(awot_ref, 0, _D, o.lanes()))

    def mha_in(c, xn):
        xn = xn.lanes()
        kt = project(bwt_ref, _D, 2 * _D, xn)
        kb = []

        def k_piece(j):
            kb.append(_pack(kt[j * 128:(j + 1) * 128, :].T))
            k_ref[j, c] = kb[j]
            if j > 0:
                low = _iota((_T // 2, 128), 1) < 64
                k_ref[_NB + j - 1, c] = jnp.where(low, kb[j], kb[j - 1])
        Lazy([lambda j=j: k_piece(j) for j in range(_NB)])

        v = project(bwt_ref, 2 * _D, 3 * _D, xn)

        def v_piece(h0):
            tail = jnp.where(_iota((_VR - _DH, _T), 0) == 0, 1.0, 0.0).astype(_F32)
            for h in range(h0, h0 + 8):
                vt_ref[c, h] = jnp.concatenate([v[h * _DH:(h + 1) * _DH, :], tail], axis=0)
        Lazy([lambda h0=h0: v_piece(h0) for h0 in range(0, _H, 8)])

        q = _pack(project(bwt_ref, 0, _D, xn) * _QSCALE)
        for j in range(_NB):
            qt_ref[c, j] = q[j * 64:(j + 1) * 64, :]
        for j in range(_NB - 1):
            qt_ref[c, _NB + j, 0:32, :] = q[(j + 1) * 64:(j + 1) * 64 + 32, :]
            qt_ref[c, _NB + j, 32:64, :] = q[j * 64 + 32:(j + 1) * 64, :]

    def lin_back_mha_front(ops, pq):
        ops = ops.get()
        o0 = lin_read(ops, pq[0])
        o1 = lin_read(ops, pq[1])
        o0.get()
        o2 = lin_read(ops, pq[2])
        xn0 = lin_out(0, o0)
        o3 = lin_read(ops, pq[3])
        xn1 = lin_out(1, o1)
        mha_in(0, xn0)
        xn2 = lin_out(2, o2)
        mha_in(1, xn1)
        xn3 = lin_out(3, o3)
        mha_in(2, xn2)
        mha_in(3, xn3)
        while pending:
            fill()

    x_cp[0].start()
    aw_cp[1].start()
    aw_cp[2].start()
    aw_cp[0].start()
    for c in range(1, _NC):
        x_cp[c].start()
    awo_cp.start()
    bw_cp.start()
    bwo_cp.start()

    def load_chunk(c):
        x_cp[c].wait()

        def piece(ls):
            xt = x_ref[c * _T + ls.start:c * _T + ls.stop, :].astype(_F32).T
            xt_ref[c, :, ls] = xt
            return _layernorm_t(xt)
        return lane_pieces(piece)

    xn = load_chunk(0).lanes()
    aw_cp[1].wait()
    transpose_weight(aw_ref, awt_ref, _NB, 2 * _NB).get()
    aw_cp[2].wait()
    wv = transpose_weight(aw_ref, awt_ref, 2 * _NB, 3 * _NB)
    pk = _blocks(_phi(project(awt_ref, _D, 2 * _D, xn)))
    wv.get()
    aw_cp[0].wait()
    wq = transpose_weight(aw_ref, awt_ref, 0, _NB)
    v = _windows(project(awt_ref, 2 * _D, 3 * _D, xn))
    wq.get()
    xn_next = load_chunk(1)
    pq = [lin_q(xn)]
    state = lin_state(None, pk, v)
    later = [(awo_cp, awo_ref, awot_ref, _NB), (bw_cp, bw_ref, bwt_ref, 3 * _NB),
             (bwo_cp, bwo_ref, bwot_ref, _NB)]
    for c in range(1, _NC):
        xn = xn_next.lanes()
        if c + 1 < _NC:
            xn_next = load_chunk(c + 1)
        cp, src, dst, n = later[c - 1]
        cp.wait()
        transpose_weight(src, dst, 0, n)
        state, q = lin_front(state, xn, last=c + 1 == _NC)
        pq.append(q)
    lin_back_mha_front(state, pq)

    for c in range(_NC):
        ot_ref[c, 0] = jnp.ones((_VR, _T), _F32)
    first_head()
    middle_heads()

    tails = [last_head(0)]
    while pending:
        fill()
    tails.append(last_head(1))
    xn0 = residual_ln(0, mha_out(0, tails[0]))
    tails.append(last_head(2))
    xn1 = residual_ln(1, mha_out(1, tails[1]))
    tails.append(last_head(3))
    state, q = lin_front(None, xn0.lanes())
    pq = [q]
    xn2 = residual_ln(2, mha_out(2, tails[2]))
    state, q = lin_front(state, xn1.lanes())
    pq.append(q)
    xn3 = residual_ln(3, mha_out(3, tails[3]))
    state, q = lin_front(state, xn2.lanes())
    pq.append(q)
    state, q = lin_front(state, xn3.lanes(), last=True)
    pq.append(q)
    lin_back_mha_front(state, pq)

    first_head()
    middle_heads()

    def store_chunk(c, xt):
        def piece(ls):
            out_ref[c * _T + ls.start:c * _T + ls.stop, :] = xt[:, ls].T.astype(_BF16)
            if ls.stop == _T:
                out_cp[c].start()
        return lane_pieces(piece)

    tails = [last_head(0)]
    while pending:
        fill()
    for c in range(_NC):
        if c + 1 < _NC:
            tails.append(last_head(c + 1))
        store_chunk(c, xt_ref[c] + mha_out(c, tails[c]))
    while pending:
        fill()
    for c in range(_NC):
        out_cp[c].wait()


@jax.jit
def pallas_interleave_layers__linear_attn_block__mha_block__prompt_kernel(
    A_x: jax.Array,
    A_wqkv: jax.Array,
    A_wo: jax.Array,
    B_x: jax.Array,
    B_wqkv: jax.Array,
    B_wo: jax.Array,
):
    del B_x
    any_spec = pl.BlockSpec(memory_space=pl.ANY)
    out = pl.pallas_call(
        _kernel,
        out_shape=jax.ShapeDtypeStruct((_S, _D), _BF16),
        in_specs=[any_spec] * 5,
        out_specs=any_spec,
        scratch_shapes=[
            pltpu.VMEM((_S, _D), _BF16),
            pltpu.VMEM((_D, 3 * _D), _BF16),
            pltpu.VMEM((_D, _D), _BF16),
            pltpu.VMEM((_D, 3 * _D), _BF16),
            pltpu.VMEM((_D, _D), _BF16),
            pltpu.VMEM((_S, _D), _BF16),
            pltpu.VMEM((_NC, _D, _T), _F32),
            pltpu.VMEM((3 * _D // 2, _D), _I32),
            pltpu.VMEM((_D // 2, _D), _I32),
            pltpu.VMEM((3 * _D // 2, _D), _I32),
            pltpu.VMEM((_D // 2, _D), _I32),
            pltpu.VMEM((_NC, 2 * _NB - 1, 64, _T), _I32),
            pltpu.VMEM((2 * _NB - 1, _NC, _T // 2, 128), _I32),
            pltpu.VMEM((_NC, _H, _VR, _T), _F32),
            pltpu.VMEM((_NC, _H, _VR, _T), _F32),
            pltpu.VMEM((_NC, _H, _VR, _T), _F32),
            pltpu.VMEM((_NC, _S, _T), _F32),
            pltpu.VMEM((_NC, 1, _T), _F32),
            pltpu.VMEM((64, _T), _I32),
            pltpu.SemaphoreType.DMA((_NC + 6,)),
            pltpu.SemaphoreType.DMA((_NC,)),
        ],
        compiler_params=pltpu.CompilerParams(vmem_limit_bytes=110 * 1024 * 1024),
    )(A_x.reshape(_S, _D), A_wqkv, A_wo, B_wqkv, B_wo)
    return out.reshape(A_x.shape)
```

```python
import math

import jax
import jax.numpy as jnp
from jax import lax
from jax.experimental import pallas as pl
from jax.experimental.pallas import tpu as pltpu

_S = 2048
_D = 640
_H = 32
_DH = _D // _H
_T = 512
_NC = _S // _T
_CK = 128
_NT = _S // _CK
_VR = 24
_NB = _D // 128
_LN_EPS = 1e-5
_QSCALE = (_DH ** -0.5) * math.log2(math.e)

_WIN = []
for _j in range(_NB):
    _lo = (128 * _j // _DH) * _DH
    _hi = -(-(128 * _j + 128) // _DH) * _DH
    _WIN.append((_lo // 16 * 16, min(_D, -(-_hi // 16) * 16)))

_F32 = jnp.float32
_BF16 = jnp.bfloat16


_I32 = jnp.int32


def _pack(x):
    return pltpu.bitcast(x.astype(_BF16), _I32)


def _operand(x):
    return pltpu.bitcast(x, _BF16) if x.dtype == _I32 else x


def _dot(a, b):
    return jnp.dot(_operand(a), _operand(b), preferred_element_type=_F32)


def _dot_nt(a, b):
    return lax.dot_general(a, b, (((1,), (1,)), ((), ())), preferred_element_type=_F32)


def _layernorm_t(x):
    mean = jnp.sum(x, axis=0, keepdims=True) * (1.0 / _D)
    d = x - mean
    var = jnp.sum(d * d, axis=0, keepdims=True) * (1.0 / _D)
    return d * lax.rsqrt(var + _LN_EPS)


def _phi(t):
    return jnp.where(t > 0, t + 1.0, jnp.exp(t)) + 1e-6


def _iota(shape, axis):
    return lax.broadcasted_iota(_I32, shape, axis)


def _kernel(x_hbm, aw_hbm, awo_hbm, bw_hbm, bwo_hbm, out_hbm,
            x_ref, aw_ref, awo_ref, bw_ref, bwo_ref, out_ref,
            xt_ref, awt_ref, bwt_ref, bwot_ref,
            qt_ref, k_ref, vt_ref, raw_ref, on_ref, s_ref, m_ref, qm_ref, in_sem, out_sem):

    def rows(c):
        return pl.ds(c * _T, _T)

    def cols(i):
        return pl.ds(i * _D, _D)

    x_cp = [pltpu.make_async_copy(x_hbm.at[rows(c)], x_ref.at[rows(c)], in_sem.at[c])
            for c in range(_NC)]
    aw_cp = [pltpu.make_async_copy(aw_hbm.at[:, cols(i)], aw_ref.at[:, cols(i)], in_sem.at[_NC + i])
             for i in range(3)]
    awo_cp = pltpu.make_async_copy(awo_hbm, awo_ref, in_sem.at[_NC + 3])
    bw_cp = pltpu.make_async_copy(bw_hbm, bw_ref, in_sem.at[_NC + 4])
    bwo_cp = pltpu.make_async_copy(bwo_hbm, bwo_ref, in_sem.at[_NC + 5])
    out_cp = [pltpu.make_async_copy(out_ref.at[pl.ds(i * 128, 128)], out_hbm.at[pl.ds(i * 128, 128)],
                                    out_sem.at[i]) for i in range(_S // 128)]

    def head_block(h):
        start = h * _DH
        off = start & 127
        return (start >> 7) + jnp.where(off > 128 - _DH, _NB, 0), off >> 1

    def masked_q(c, jb, off2):
        keep = ((_iota((64, _T), 0) - off2) & 63) < _DH // 2
        return jnp.where(keep, qt_ref[c, jb], 0)

    def scores(jb, qm, t):
        cc, r0 = divmod(t * _CK, _T)
        return _dot(k_ref[jb, cc, r0 // 2:(r0 + _CK) // 2, :], qm)

    def tile_max(mx, s):
        cm = jnp.max(s.reshape(_CK // 8, 8, _T), axis=0)
        return cm if mx is None else jnp.maximum(mx, cm)

    def weigh(acc, h, t, s, m):
        cc, r0 = divmod(t * _CK, _T)
        ov = _dot(vt_ref[cc, h, :, r0:r0 + _CK], jnp.exp2(s - m))
        return ov if acc is None else acc + ov

    def normalise(acc):
        return acc * (1.0 / acc[_DH:_DH + 1, :])

    def tile(t):
        return slice(t * _CK, (t + 1) * _CK)

    def stage_q(h):
        jb, off2 = head_block(h)
        qm_ref[...] = masked_q(0, jb, off2)
        return jb, off2

    def first_head():
        jb, off2 = head_block(0)
        for c in range(_NC):
            qm = masked_q(c, jb, off2)
            mx = None
            for t in range(_NT):
                s = scores(jb, qm, t)
                s_ref[c, tile(t), :] = s
                mx = tile_max(mx, s)
            m_ref[c] = jnp.max(mx, axis=0, keepdims=True)

    def middle_heads():
        def body(h, carry):
            jb, off2 = carry
            for c in range(_NC):
                on_ref[c, h] = normalise(raw_ref[c, h])
            for c in range(_NC):
                qm = qm_ref[...] if c == 0 else masked_q(c, jb, off2)
                m = m_ref[c]
                mx = acc = None
                for t in range(_NT):
                    old = s_ref[c, tile(t), :]
                    s = scores(jb, qm, t)
                    s_ref[c, tile(t), :] = s
                    mx = tile_max(mx, s)
                    acc = weigh(acc, h, t, old, m)
                raw_ref[c, h + 1] = acc
                m_ref[c] = jnp.max(mx, axis=0, keepdims=True)
            return stage_q(h + 2)
        for c in range(_NC):
            raw_ref[c, 0] = jnp.ones((_VR, _T), _F32)
        lax.fori_loop(0, _H - 2, body, stage_q(1))

    def last_heads():
        jb, off2 = head_block(_H - 1)
        outs = []
        prev = None
        for c in range(_NC):
            qm = qm_ref[...] if c == 0 else masked_q(c, jb, off2)
            mx = acc = last = None
            tiles = []
            for t in range(_NT):
                s = scores(jb, qm, t)
                tiles.append(s)
                mx = tile_max(mx, s)
                acc = weigh(acc, _H - 2, t, s_ref[c, tile(t), :], m_ref[c])
                if prev is not None:
                    last = weigh(last, _H - 1, t, prev[0][t], prev[1])
            if prev is not None:
                outs[-1].append(last)
            outs.append([acc])
            prev = (tiles, jnp.max(mx, axis=0, keepdims=True))

        def piece(t0):
            acc = None
            for t in range(t0, t0 + 2):
                acc = weigh(acc, _H - 1, t, prev[0][t], prev[1])
            return acc
        outs[-1].append(Lazy([lambda t0=t0: piece(t0) for t0 in range(0, _NT, 2)]))
        return outs

    pending = []

    class Lazy:
        def __init__(self, pieces):
            self.pieces = list(pieces)
            self.values = []
            pending.append(self)

        def step(self):
            self.values.append(self.pieces[len(self.values)]())
            if len(self.values) == len(self.pieces):
                pending.remove(self)

        def get(self):
            while len(self.values) < len(self.pieces):
                self.step()
            return self.values

        def lanes(self):
            return jnp.concatenate(self.get(), axis=1).astype(_BF16)

    def fill():
        for lazy in list(pending):
            lazy.step()

    def project(w_ref, lo, hi, rhs, rows_per_piece=128):
        outs = []
        for r in range(lo, hi, rows_per_piece):
            outs.append(_dot(w_ref[r // 2:(r + rows_per_piece) // 2, :], rhs))
            fill()
        return jnp.concatenate(outs, axis=0)

    def lane_pieces(fn):
        return Lazy([lambda i=i: fn(slice(i * 128, (i + 1) * 128)) for i in range(_T // 128)])

    def transpose_weight(src, dst, lo, hi):
        def piece(j):
            dst[j * 64:(j + 1) * 64, :] = _pack(src[:, j * 128:(j + 1) * 128].astype(_F32).T)
        return Lazy([lambda j=j: piece(j) for j in range(lo, hi)])

    def residual_ln(c, delta):
        xt = xt_ref[c] + delta
        xt_ref[c] = xt
        return lane_pieces(lambda ls: _layernorm_t(xt[:, ls]))

    def mha_out(c, tail):
        acc30, acc31 = tail
        if isinstance(acc31, Lazy):
            parts = acc31.get()
            acc31 = parts[0]
            for p in parts[1:]:
                acc31 = acc31 + p
        heads = [on_ref[c, h + 1, 0:_DH, :] for h in range(_H - 3)]
        heads += [normalise(a)[0:_DH, :] for a in (raw_ref[c, _H - 2], acc30, acc31)]
        return project(bwot_ref, 0, _D, jnp.concatenate(heads, axis=0).astype(_BF16))

    def lin_front(state, xn, q_rows=_D):
        pk = _phi(project(awt_ref, _D, 2 * _D, xn))
        z = pk[:, 0:128]
        for i in range(1, _T // 128):
            z = z + pk[:, i * 128:(i + 1) * 128]
        pq = _phi(project(awt_ref, 0, 128, xn))
        g = _dot_nt(pk.astype(_BF16), xn)
        if q_rows > 128:
            pq = jnp.concatenate([pq, _phi(project(awt_ref, 128, q_rows, xn))], axis=0)
        return ((z, g) if state is None else (state[0] + z, state[1] + g)), pq

    def head_of(i):
        return (i * 3277) >> 16

    def lin_operands(state, cover):
        z, g = state
        cover()
        kv = [_dot(g[lo:hi, :].astype(_BF16), aw_ref[:, 2 * _D + j * 128:2 * _D + (j + 1) * 128])
              for j, (lo, hi) in enumerate(_WIN)]
        cover()
        parts = []
        for j, (lo, hi) in enumerate(_WIN):
            same = head_of(_iota((hi - lo, 128), 0) + lo) == head_of(_iota((1, 128), 1) + 128 * j)
            parts.append(_dot(_pack(jnp.where(same, kv[j], 0.0)), awo_ref[j * 128:(j + 1) * 128, :]))
        edges = sorted({e for w in _WIN for e in w})
        rows_out = []
        for a, b in zip(edges[:-1], edges[1:]):
            acc = None
            for j, (lo, hi) in enumerate(_WIN):
                if lo <= a and b <= hi:
                    part = parts[j][a - lo:b - lo, :]
                    acc = part if acc is None else acc + part
            rows_out.append(acc)
        mt = _pack(jnp.concatenate(rows_out, axis=0).T)
        zcol = jnp.broadcast_to(jnp.sum(z, axis=1, keepdims=True), (_D, 128))
        zrow = jnp.concatenate([zcol[j * 128:(j + 1) * 128, :].T[0:_H, :] for j in range(_NB)], axis=1)
        zc = jnp.where(_iota((_H, _D), 0) == head_of(_iota((1, _D), 1)), zrow, 0.0)
        return _pack(zc), mt

    def lin_scale(zc, pq):
        den = _dot(zc, pq.astype(_BF16))

        def piece(ls):
            inv = 1.0 / (den[:, ls] + 1e-6)
            sub = _iota((8, 128), 0)
            groups = []
            for a in range(0, _D, 8):
                h = a // _DH
                scale = jnp.broadcast_to(inv[h:h + 1, :], (8, 128))
                split = (h + 1) * _DH - a
                if split < 8:
                    scale = jnp.where(sub < split, scale, jnp.broadcast_to(inv[h + 1:h + 2, :], (8, 128)))
                groups.append(pq[a:a + 8, ls] * scale)
            return jnp.concatenate(groups, axis=0)
        return lane_pieces(piece)

    def lin_out(c, mt, q):
        return residual_ln(c, project(mt, 0, _D, q.lanes()))

    def mha_in(c, xn):
        xn = xn.lanes()
        kt = project(bwt_ref, _D, 2 * _D, xn)
        kb = []

        def k_piece(j):
            kb.append(_pack(kt[j * 128:(j + 1) * 128, :].T))
            k_ref[j, c] = kb[j]
            if j > 0:
                low = _iota((_T // 2, 128), 1) < 64
                k_ref[_NB + j - 1, c] = jnp.where(low, kb[j], kb[j - 1])
        Lazy([lambda j=j: k_piece(j) for j in range(_NB)])

        v = project(bwt_ref, 2 * _D, 3 * _D, xn)

        def v_piece(h0):
            tail = jnp.where(_iota((_VR - _DH, _T), 0) == 0, 1.0, 0.0).astype(_F32)
            for h in range(h0, h0 + 8):
                vt_ref[c, h] = jnp.concatenate([v[h * _DH:(h + 1) * _DH, :], tail], axis=0)
        Lazy([lambda h0=h0: v_piece(h0) for h0 in range(0, _H, 8)])

        q = _pack(project(bwt_ref, 0, _D, xn) * _QSCALE)
        for j in range(_NB):
            qt_ref[c, j] = q[j * 64:(j + 1) * 64, :]
        for j in range(_NB - 1):
            qt_ref[c, _NB + j, 0:32, :] = q[(j + 1) * 64:(j + 1) * 64 + 32, :]
            qt_ref[c, _NB + j, 32:64, :] = q[j * 64 + 32:(j + 1) * 64, :]

    def lin_back_mha_front(state, pq, xn_last):
        state, q_parts = lin_front(state, xn_last, 128)
        q_parts = [q_parts]

        def cover():
            r = 128 * len(q_parts)
            q_parts.append(_phi(project(awt_ref, r, r + 128, xn_last)))

        zc, mt = lin_operands(state, cover)
        q0 = lin_scale(zc, pq[0])
        q1 = lin_scale(zc, pq[1])
        cover()
        q2 = lin_scale(zc, pq[2])
        cover()
        q3 = lin_scale(zc, jnp.concatenate(q_parts, axis=0))
        xn0 = lin_out(0, mt, q0)
        xn1 = lin_out(1, mt, q1)
        mha_in(0, xn0)
        xn2 = lin_out(2, mt, q2)
        mha_in(1, xn1)
        xn3 = lin_out(3, mt, q3)
        mha_in(2, xn2)
        mha_in(3, xn3)
        while pending:
            fill()

    x_cp[0].start()
    aw_cp[1].start()

    def load_chunk(c):
        x_cp[c].wait()

        def piece(ls):
            xt = x_ref[c * _T + ls.start:c * _T + ls.stop, :].astype(_F32).T
            xt_ref[c, :, ls] = xt
            return _layernorm_t(xt)
        return lane_pieces(piece)

    xn = load_chunk(0)
    aw_cp[0].start()
    xn = xn.lanes()
    aw_cp[1].wait()
    for c in range(1, _NC):
        x_cp[c].start()
    transpose_weight(aw_ref, awt_ref, _NB, 2 * _NB).get()
    aw_cp[0].wait()
    for cp in (bw_cp, bwo_cp, aw_cp[2], awo_cp):
        cp.start()
    transpose_weight(aw_ref, awt_ref, 0, _NB)
    state, pq = None, []
    for c in range(_NC - 1):
        xn_next = load_chunk(c + 1)
        if c == 1:
            bw_cp.wait()
            transpose_weight(bw_ref, bwt_ref, 0, 3 * _NB)
        if c == 2:
            bwo_cp.wait()
            transpose_weight(bwo_ref, bwot_ref, 0, _NB)
            aw_cp[2].wait()
            awo_cp.wait()
        state, q = lin_front(state, xn)
        pq.append(q)
        xn = xn_next.lanes()
    lin_back_mha_front(state, pq, xn)

    first_head()
    middle_heads()

    tails = last_heads()
    xn0 = residual_ln(0, mha_out(0, tails[0]))
    xn1 = residual_ln(1, mha_out(1, tails[1]))
    state, q = lin_front(None, xn0.lanes())
    pq = [q]
    xn2 = residual_ln(2, mha_out(2, tails[2]))
    state, q = lin_front(state, xn1.lanes())
    pq.append(q)
    xn3 = residual_ln(3, mha_out(3, tails[3]))
    state, q = lin_front(state, xn2.lanes())
    pq.append(q)
    lin_back_mha_front(state, pq, xn3.lanes())

    first_head()
    middle_heads()

    def store_chunk(c, xt):
        def piece(ls):
            out_ref[c * _T + ls.start:c * _T + ls.stop, :] = xt[:, ls].T.astype(_BF16)
            out_cp[(c * _T + ls.start) // 128].start()
        return lane_pieces(piece)

    tails = last_heads()
    for c in range(_NC):
        store_chunk(c, xt_ref[c] + mha_out(c, tails[c]))
    while pending:
        fill()
    for cp in out_cp:
        cp.wait()


@jax.jit
def pallas_interleave_layers__linear_attn_block__mha_block__prompt_kernel(
    A_x: jax.Array,
    A_wqkv: jax.Array,
    A_wo: jax.Array,
    B_x: jax.Array,
    B_wqkv: jax.Array,
    B_wo: jax.Array,
):
    del B_x
    any_spec = pl.BlockSpec(memory_space=pl.ANY)
    out = pl.pallas_call(
        _kernel,
        out_shape=jax.ShapeDtypeStruct((_S, _D), _BF16),
        in_specs=[any_spec] * 5,
        out_specs=any_spec,
        scratch_shapes=[
            pltpu.VMEM((_S, _D), _BF16),
            pltpu.VMEM((_D, 3 * _D), _BF16),
            pltpu.VMEM((_D, _D), _BF16),
            pltpu.VMEM((_D, 3 * _D), _BF16),
            pltpu.VMEM((_D, _D), _BF16),
            pltpu.VMEM((_S, _D), _BF16),
            pltpu.VMEM((_NC, _D, _T), _F32),
            pltpu.VMEM((_D, _D), _I32),
            pltpu.VMEM((3 * _D // 2, _D), _I32),
            pltpu.VMEM((_D // 2, _D), _I32),
            pltpu.VMEM((_NC, 2 * _NB - 1, 64, _T), _I32),
            pltpu.VMEM((2 * _NB - 1, _NC, _T // 2, 128), _I32),
            pltpu.VMEM((_NC, _H, _VR, _T), _F32),
            pltpu.VMEM((_NC, _H - 1, _VR, _T), _F32),
            pltpu.VMEM((_NC, _H - 2, _VR, _T), _F32),
            pltpu.VMEM((_NC, _S, _T), _F32),
            pltpu.VMEM((_NC, 1, _T), _F32),
            pltpu.VMEM((64, _T), _I32),
            pltpu.SemaphoreType.DMA((_NC + 6,)),
            pltpu.SemaphoreType.DMA((_S // 128,)),
        ],
        compiler_params=pltpu.CompilerParams(vmem_limit_bytes=110 * 1024 * 1024),
    )(A_x.reshape(_S, _D), A_wqkv, A_wo, B_wqkv, B_wo)
    return out.reshape(A_x.shape)
```

```python
import math

import jax
import jax.numpy as jnp
from jax import lax
from jax.experimental import pallas as pl
from jax.experimental.pallas import tpu as pltpu

_S = 2048
_D = 640
_H = 32
_DH = _D // _H
_T = 512
_NC = _S // _T
_CK = 128
_NT = _S // _CK
_VR = 24
_NB = _D // 128
_LN_EPS = 1e-5
_QSCALE = (_DH ** -0.5) * math.log2(math.e)

_WIN = []
for _j in range(_NB):
    _lo = (128 * _j // _DH) * _DH
    _hi = -(-(128 * _j + 128) // _DH) * _DH
    _WIN.append((_lo // 16 * 16, min(_D, -(-_hi // 16) * 16)))

_F32 = jnp.float32
_BF16 = jnp.bfloat16
_I32 = jnp.int32


def _pack(x):
    return pltpu.bitcast(x.astype(_BF16), _I32)


def _operand(x):
    return pltpu.bitcast(x, _BF16) if x.dtype == _I32 else x


def _dot(a, b):
    return jnp.dot(_operand(a), _operand(b), precision=lax.Precision.DEFAULT,
                   preferred_element_type=_F32)


def _dot_nt(a, b):
    return lax.dot_general(a, b, (((1,), (1,)), ((), ())), precision=lax.Precision.DEFAULT,
                           preferred_element_type=_F32)


def _layernorm_t(x):
    mean = jnp.sum(x, axis=0, keepdims=True) * (1.0 / _D)
    d = x - mean
    var = jnp.sum(d * d, axis=0, keepdims=True) * (1.0 / _D)
    return d * lax.rsqrt(var + _LN_EPS)


def _phi(t):
    return jnp.where(t > 0, t + 1.0, jnp.exp(t)) + 1e-6


def _iota(shape, axis):
    return lax.broadcasted_iota(_I32, shape, axis)


def _kernel(x_hbm, aw_hbm, awo_hbm, bw_hbm, bwo_hbm, out_hbm,
            x_ref, aw_ref, awo_ref, bw_ref, bwo_ref, out_ref,
            xt_ref, awt_ref, bwt_ref, bwot_ref,
            qt_ref, k_ref, vt_ref, raw_ref, on_ref, s_ref, m_ref, qm_ref, fence_ref, in_sem, out_sem):

    n_sems = [0]

    def copy_in(src, dst, row0, n_rows, col0=0, n_cols=None):
        idx = (pl.ds(row0, n_rows), pl.ds(col0, n_cols or src.shape[1]))
        n_sems[0] += 1
        return pltpu.make_async_copy(src.at[idx], dst.at[idx], in_sem.at[n_sems[0] - 1])

    x_cp = [copy_in(x_hbm, x_ref, c * _T, _T) for c in range(_NC)]
    aq_cp = [copy_in(aw_hbm, aw_ref, 0, _D, 0, 256), copy_in(aw_hbm, aw_ref, 0, _D, 256, _D - 256)]
    ak_cp = copy_in(aw_hbm, aw_ref, 0, _D, _D, _D)
    av_cp = copy_in(aw_hbm, aw_ref, 0, _D, 2 * _D, _D)
    awo_cp = copy_in(awo_hbm, awo_ref, 0, _D)
    bw_cp = copy_in(bw_hbm, bw_ref, 0, _D)
    bwo_cp = copy_in(bwo_hbm, bwo_ref, 0, _D)
    fence_cp = copy_in(x_hbm, fence_ref, 0, 16)
    out_cp = [pltpu.make_async_copy(out_ref.at[pl.ds(i * 128, 128)], out_hbm.at[pl.ds(i * 128, 128)],
                                    out_sem.at[i]) for i in range(_S // 128)]

    def head_block(h):
        start = h * _DH
        off = start & 127
        return (start >> 7) + jnp.where(off > 128 - _DH, _NB, 0), off >> 1

    def masked_q(c, jb, off2):
        keep = ((_iota((64, _T), 0) - off2) & 63) < _DH // 2
        return jnp.where(keep, qt_ref[c, jb], 0)

    def scores(jb, qm, t):
        cc, r0 = divmod(t * _CK, _T)
        return _dot(k_ref[jb, cc, r0 // 2:(r0 + _CK) // 2, :], qm)

    def tile_max(mx, s):
        cm = jnp.max(s.reshape(_CK // 8, 8, _T), axis=0)
        return cm if mx is None else jnp.maximum(mx, cm)

    def weigh(acc, h, t, s, m):
        cc, r0 = divmod(t * _CK, _T)
        ov = _dot(vt_ref[cc, h, :, r0:r0 + _CK], jnp.exp2(s - m))
        return ov if acc is None else acc + ov

    def normalise(acc):
        return acc * (1.0 / acc[_DH:_DH + 1, :])

    def tile(t):
        return slice(t * _CK, (t + 1) * _CK)

    def stage_q(h):
        jb, off2 = head_block(h)
        qm_ref[...] = masked_q(0, jb, off2)
        return jb, off2

    def first_head():
        jb, off2 = head_block(0)
        for c in range(_NC):
            qm = masked_q(c, jb, off2)
            mx = None
            for t in range(_NT):
                s = scores(jb, qm, t)
                s_ref[c, tile(t), :] = s
                mx = tile_max(mx, s)
            m_ref[c] = jnp.max(mx, axis=0, keepdims=True)

    def middle_heads():
        def body(h, carry):
            jb, off2 = carry
            for c in range(_NC):
                on_ref[c, h] = normalise(raw_ref[c, h])
            for c in range(_NC):
                qm = qm_ref[...] if c == 0 else masked_q(c, jb, off2)
                m = m_ref[c]
                mx = acc = None
                for t in range(_NT):
                    old = s_ref[c, tile(t), :]
                    s = scores(jb, qm, t)
                    s_ref[c, tile(t), :] = s
                    mx = tile_max(mx, s)
                    acc = weigh(acc, h, t, old, m)
                raw_ref[c, h + 1] = acc
                m_ref[c] = jnp.max(mx, axis=0, keepdims=True)
            return stage_q(h + 2)
        for c in range(_NC):
            raw_ref[c, 0] = jnp.ones((_VR, _T), _F32)
        lax.fori_loop(0, _H - 2, body, stage_q(1))

    def last_heads():
        jb, off2 = head_block(_H - 1)
        outs = []
        prev = None
        for c in range(_NC):
            qm = qm_ref[...] if c == 0 else masked_q(c, jb, off2)
            mx = acc = last = None
            tiles = []
            for t in range(_NT):
                s = scores(jb, qm, t)
                tiles.append(s)
                mx = tile_max(mx, s)
                acc = weigh(acc, _H - 2, t, s_ref[c, tile(t), :], m_ref[c])
                if prev is not None:
                    last = weigh(last, _H - 1, t, prev[0][t], prev[1])
            if prev is not None:
                outs[-1].append(last)
            outs.append([acc])
            prev = (tiles, jnp.max(mx, axis=0, keepdims=True))

        def piece(t0):
            acc = None
            for t in range(t0, t0 + 2):
                acc = weigh(acc, _H - 1, t, prev[0][t], prev[1])
            return acc
        outs[-1].append(Lazy([lambda t0=t0: piece(t0) for t0 in range(0, _NT, 2)]))
        return outs

    pending = []

    class Lazy:
        def __init__(self, pieces):
            self.pieces = list(pieces)
            self.values = []
            pending.append(self)

        def step(self):
            self.values.append(self.pieces[len(self.values)]())
            if len(self.values) == len(self.pieces):
                pending.remove(self)

        def get(self):
            while len(self.values) < len(self.pieces):
                self.step()
            return self.values

        def lanes(self):
            return jnp.concatenate(self.get(), axis=1).astype(_BF16)

    def fill():
        for lazy in list(pending):
            lazy.step()

    fine = [True]

    def project(w_ref, lo, hi, rhs):
        step = 128 if fine[0] else hi - lo
        outs = []
        for r in range(lo, hi, step):
            outs.append(_dot(w_ref[r // 2:(r + step) // 2, :], rhs))
            fill()
        return jnp.concatenate(outs, axis=0)

    def lane_pieces(fn):
        return Lazy([lambda i=i: fn(slice(i * 128, (i + 1) * 128)) for i in range(_T // 128)])

    def transpose_weight(src, dst, lo, hi):
        for j in range(lo, hi):
            dst[j * 64:(j + 1) * 64, :] = _pack(src[:, j * 128:(j + 1) * 128].astype(_F32).T)

    def residual_ln(c, delta):
        xt = xt_ref[c] + delta
        xt_ref[c] = xt
        return lane_pieces(lambda ls: _layernorm_t(xt[:, ls]))

    def mha_out(c, tail):
        acc30, acc31 = tail
        if isinstance(acc31, Lazy):
            parts = acc31.get()
            acc31 = parts[0]
            for p in parts[1:]:
                acc31 = acc31 + p
        heads = [on_ref[c, h + 1, 0:_DH, :] for h in range(_H - 3)]
        heads += [normalise(a)[0:_DH, :] for a in (raw_ref[c, _H - 2], acc30, acc31)]
        return project(bwot_ref, 0, _D, jnp.concatenate(heads, axis=0).astype(_BF16))

    class LinFront:
        def __init__(self, xn):
            self.xn = xn.lanes()
            self.q_parts, self.q_rows, self.pk = [], 0, None

        def q(self, upto=_D):
            self.q_parts.append(_phi(project(awt_ref, self.q_rows, upto, self.xn)))
            self.q_rows = upto

        def k(self, midway=None):
            parts = []
            if midway is not None:
                parts.append(project(awt_ref, _D, _D + 256, self.xn))
                midway()
            parts.append(project(awt_ref, _D + 256 * len(parts), 2 * _D, self.xn))
            self.pk = _phi(jnp.concatenate(parts, axis=0))

        def accumulate(self, state):
            z = self.pk[:, 0:128]
            for i in range(1, _T // 128):
                z = z + self.pk[:, i * 128:(i + 1) * 128]
            g = _dot_nt(self.pk.astype(_BF16), self.xn)
            return (z, g) if state is None else (state[0] + z, state[1] + g)

        def all(self, state, midway=None):
            self.k(midway)
            self.q(self.q_rows + 128)
            state = self.accumulate(state)
            self.q()
            return state

        def pq(self):
            return jnp.concatenate(self.q_parts, axis=0)

    def head_of(i):
        return (i * 3277) >> 16

    def lin_operands(state, cover):
        z, g = state
        cover()
        kv = [_dot(g[lo:hi, :].astype(_BF16), aw_ref[:, 2 * _D + j * 128:2 * _D + (j + 1) * 128])
              for j, (lo, hi) in enumerate(_WIN)]
        cover()
        parts = []
        for j, (lo, hi) in enumerate(_WIN):
            same = head_of(_iota((hi - lo, 128), 0) + lo) == head_of(_iota((1, 128), 1) + 128 * j)
            parts.append(_dot(_pack(jnp.where(same, kv[j], 0.0)), awo_ref[j * 128:(j + 1) * 128, :]))
        edges = sorted({e for w in _WIN for e in w})
        rows_out = []
        for a, b in zip(edges[:-1], edges[1:]):
            acc = None
            for j, (lo, hi) in enumerate(_WIN):
                if lo <= a and b <= hi:
                    part = parts[j][a - lo:b - lo, :]
                    acc = part if acc is None else acc + part
            rows_out.append(acc)
        mt = _pack(jnp.concatenate(rows_out, axis=0).T)
        zcol = jnp.broadcast_to(jnp.sum(z, axis=1, keepdims=True), (_D, 128))
        zrow = jnp.concatenate([zcol[j * 128:(j + 1) * 128, :].T[0:_H, :] for j in range(_NB)], axis=1)
        zc = jnp.where(_iota((_H, _D), 0) == head_of(_iota((1, _D), 1)), zrow, 0.0)
        return _pack(zc), mt

    def lin_scale(zc, pq):
        den = _dot(zc, pq.astype(_BF16))

        def piece(ls):
            inv = 1.0 / (den[:, ls] + 1e-6)
            sub = _iota((8, 128), 0)
            groups = []
            for a in range(0, _D, 8):
                h = a // _DH
                scale = jnp.broadcast_to(inv[h:h + 1, :], (8, 128))
                split = (h + 1) * _DH - a
                if split < 8:
                    scale = jnp.where(sub < split, scale, jnp.broadcast_to(inv[h + 1:h + 2, :], (8, 128)))
                groups.append(pq[a:a + 8, ls] * scale)
            return jnp.concatenate(groups, axis=0)
        return lane_pieces(piece)

    def lin_out(c, mt, q):
        return residual_ln(c, project(mt, 0, _D, q.lanes()))

    def mha_in(c, xn):
        xn = xn.lanes()
        kt = project(bwt_ref, _D, 2 * _D, xn)
        kb = []

        def k_piece(j):
            kb.append(_pack(kt[j * 128:(j + 1) * 128, :].T))
            k_ref[j, c] = kb[j]
            if j > 0:
                low = _iota((_T // 2, 128), 1) < 64
                k_ref[_NB + j - 1, c] = jnp.where(low, kb[j], kb[j - 1])
        Lazy([lambda j=j: k_piece(j) for j in range(_NB)])

        v = project(bwt_ref, 2 * _D, 3 * _D, xn)

        def v_piece(h0):
            tail = jnp.where(_iota((_VR - _DH, _T), 0) == 0, 1.0, 0.0).astype(_F32)
            for h in range(h0, h0 + 8):
                vt_ref[c, h] = jnp.concatenate([v[h * _DH:(h + 1) * _DH, :], tail], axis=0)
        Lazy([lambda h0=h0: v_piece(h0) for h0 in range(0, _H, 8)])

        q = _pack(project(bwt_ref, 0, _D, xn) * _QSCALE)
        for j in range(_NB):
            qt_ref[c, j] = q[j * 64:(j + 1) * 64, :]
        for j in range(_NB - 1):
            qt_ref[c, _NB + j, 0:32, :] = q[(j + 1) * 64:(j + 1) * 64 + 32, :]
            qt_ref[c, _NB + j, 32:64, :] = q[j * 64 + 32:(j + 1) * 64, :]

    def lin_back_mha_front(state, fronts):
        last = fronts[-1]

        def cover():
            last.q(last.q_rows + 128)

        last.k()
        cover()
        zc, mt = lin_operands(last.accumulate(state), cover)
        q0 = lin_scale(zc, fronts[0].pq())
        q1 = lin_scale(zc, fronts[1].pq())
        cover()
        q2 = lin_scale(zc, fronts[2].pq())
        cover()
        q3 = lin_scale(zc, last.pq())
        xn0 = lin_out(0, mt, q0)
        xn1 = lin_out(1, mt, q1)
        mha_in(0, xn0)
        xn2 = lin_out(2, mt, q2)
        mha_in(1, xn1)
        xn3 = lin_out(3, mt, q3)
        mha_in(2, xn2)
        mha_in(3, xn3)
        while pending:
            fill()

    for cp in (x_cp[0], aq_cp[0], aq_cp[1], ak_cp, x_cp[1]):
        cp.start()

    def load_chunk(c):
        x_cp[c].wait()

        def piece(ls):
            xt = x_ref[c * _T + ls.start:c * _T + ls.stop, :].astype(_F32).T
            xt_ref[c, :, ls] = xt
            return _layernorm_t(xt)
        return lane_pieces(piece)

    nxt = []
    later = [av_cp, awo_cp, bw_cp, bwo_cp]

    def arrive(chunk):
        def hook():
            if chunk == _NC - 1:
                for cp in later:
                    cp.wait()
            nxt.append(load_chunk(chunk))
            if chunk == 1:
                for cp in x_cp[2:] + later + [fence_cp]:
                    cp.start()
            if chunk == _NC - 1:
                transpose_weight(bw_ref, bwt_ref, 0, 3 * _NB)
                transpose_weight(bwo_ref, bwot_ref, 0, _NB)
        return hook

    fronts = [LinFront(load_chunk(0))]
    aq_cp[0].wait()
    transpose_weight(aw_ref, awt_ref, 0, 2)
    fronts[0].q(256)
    aq_cp[1].wait()
    transpose_weight(aw_ref, awt_ref, 2, _NB)
    fronts[0].q()
    ak_cp.wait()
    transpose_weight(aw_ref, awt_ref, _NB, 2 * _NB)
    fronts[0].k(arrive(1))
    fine[0] = False
    fronts.append(LinFront(nxt[0]))
    fronts[1].q(128)
    state = fronts[0].accumulate(None)
    state = fronts[1].all(state, arrive(2))
    fronts.append(LinFront(nxt[1]))
    state = fronts[2].all(state, arrive(3))
    fronts.append(LinFront(nxt[2]))
    lin_back_mha_front(state, fronts)

    first_head()
    middle_heads()

    tails = last_heads()
    fine[0] = True
    xn0 = residual_ln(0, mha_out(0, tails[0]))
    xn1 = residual_ln(1, mha_out(1, tails[1]))
    fine[0] = False
    fronts = [LinFront(xn0)]
    state = fronts[0].all(None)
    xn2 = residual_ln(2, mha_out(2, tails[2]))
    fronts.append(LinFront(xn1))
    state = fronts[1].all(state)
    xn3 = residual_ln(3, mha_out(3, tails[3]))
    fronts.append(LinFront(xn2))
    state = fronts[2].all(state)
    fronts.append(LinFront(xn3))
    lin_back_mha_front(state, fronts)

    first_head()
    middle_heads()

    def store_chunk(c, xt):
        def piece(ls):
            out_ref[c * _T + ls.start:c * _T + ls.stop, :] = xt[:, ls].T.astype(_BF16)
            out_cp[(c * _T + ls.start) // 128].start()
        return lane_pieces(piece)

    tails = last_heads()
    for c in range(_NC):
        fine[0] = c < 2
        xt = xt_ref[c] + mha_out(c, tails[c])
        while c > 0 and pending:
            fill()
        if c == 1:
            fence_cp.wait()
        if c == 2:
            for cp in out_cp[0:4]:
                cp.wait()
        store_chunk(c, xt)
    while pending:
        fill()
    for cp in out_cp[4:]:
        cp.wait()


@jax.jit
def pallas_interleave_layers__linear_attn_block__mha_block__prompt_kernel(
    A_x: jax.Array,
    A_wqkv: jax.Array,
    A_wo: jax.Array,
    B_x: jax.Array,
    B_wqkv: jax.Array,
    B_wo: jax.Array,
):
    del B_x
    any_spec = pl.BlockSpec(memory_space=pl.ANY)
    out = pl.pallas_call(
        _kernel,
        out_shape=jax.ShapeDtypeStruct((_S, _D), _BF16),
        in_specs=[any_spec] * 5,
        out_specs=any_spec,
        scratch_shapes=[
            pltpu.VMEM((_S, _D), _BF16),
            pltpu.VMEM((_D, 3 * _D), _BF16),
            pltpu.VMEM((_D, _D), _BF16),
            pltpu.VMEM((_D, 3 * _D), _BF16),
            pltpu.VMEM((_D, _D), _BF16),
            pltpu.VMEM((_S, _D), _BF16),
            pltpu.VMEM((_NC, _D, _T), _F32),
            pltpu.VMEM((_D, _D), _I32),
            pltpu.VMEM((3 * _D // 2, _D), _I32),
            pltpu.VMEM((_D // 2, _D), _I32),
            pltpu.VMEM((_NC, 2 * _NB - 1, 64, _T), _I32),
            pltpu.VMEM((2 * _NB - 1, _NC, _T // 2, 128), _I32),
            pltpu.VMEM((_NC, _H, _VR, _T), _F32),
            pltpu.VMEM((_NC, _H - 1, _VR, _T), _F32),
            pltpu.VMEM((_NC, _H - 2, _VR, _T), _F32),
            pltpu.VMEM((_NC, _S, _T), _F32),
            pltpu.VMEM((_NC, 1, _T), _F32),
            pltpu.VMEM((64, _T), _I32),
            pltpu.VMEM((16, _D), _BF16),
            pltpu.SemaphoreType.DMA((_NC + 8,)),
            pltpu.SemaphoreType.DMA((_S // 128,)),
        ],
        compiler_params=pltpu.CompilerParams(vmem_limit_bytes=110 * 1024 * 1024),
    )(A_x.reshape(_S, _D), A_wqkv, A_wo, B_wqkv, B_wo)
    return out.reshape(A_x.shape)
```
